```python
import jax
import jax.numpy as jnp

def _softmax(x, axis=-1):
    return jax.nn.softmax(x, axis=axis)
def _gelu(x):
    return jax.nn.gelu(x, approximate=True)
def _silu(x):
    return jax.nn.silu(x)
def _sigmoid(x):
    return jax.nn.sigmoid(x)
def _layernorm(x, axis=-1, eps=1e-5):
    m = jnp.mean(x, axis=axis, keepdims=True)
    v = jnp.var(x, axis=axis, keepdims=True)
    return (x - m) / jnp.sqrt(v + eps)
def _scatter_add(tgt, idx, src, axis=0):
    return tgt.at[idx].add(src)
def _segment_sum(src, seg, n):
    return jax.ops.segment_sum(src, seg, n)
class _Rng:
    def __init__(self, key):
        self._k = key
    def _next(self):
        self._k, sub = jax.random.split(self._k)
        return sub
    def normal(self, shape):
        return jax.random.normal(self._next(), shape, dtype=jnp.bfloat16)
    def randint(self, lo, hi, shape):
        return jax.random.randint(self._next(), shape, lo, hi, dtype=jnp.int32)
    def uniform(self, shape, lo=0.0, hi=1.0):
        return jax.random.uniform(self._next(), shape, jnp.bfloat16, lo, hi)
    def permutation(self, n):
        return jax.random.permutation(self._next(), n)


kernel_name = 'standalone__modern_conv_block_convnext__vision'

def setup_inputs():
    _rng = _Rng(jax.random.key(int.from_bytes(__import__("os").urandom(4), "little")))
    _w = (lambda a: (lambda t: t.astype(jnp.bfloat16) if jnp.issubdtype(t.dtype, jnp.floating) else t)(jnp.asarray(a)))
    H = W = 512
    C = 96
    K = 3
    return {
        "x": _w((lambda *s: _rng.normal(s) * 0.05)(1, H, W, C)),
        "dw": _w((lambda *s: _rng.normal(s) * 0.05)(K, K, C)),
        "w1": _w((lambda *s: _rng.normal(s) * 0.05)(C, 4 * C)),
        "b1": _w((lambda *s: _rng.normal(s) * 0.05)(4 * C)),
        "w2": _w((lambda *s: _rng.normal(s) * 0.05)(4 * C, C)),
        "b2": _w((lambda *s: _rng.normal(s) * 0.05)(C)),
        "gamma": _w((lambda *s: _rng.normal(s) * 0.05)(C)),
    }

def reference(x, dw, w1, b1, w2, b2, gamma):
    B, H, W, C = x.shape
    K = dw.shape[0]
    pad = K // 2
    xp = jnp.pad(x, ((0,0),(pad,pad),(pad,pad),(0,0)))
    out = jnp.zeros_like(x)
    for i in range(K):
        for j in range(K):
            out = out + xp[:, i:i+H, j:j+W, :] * dw[i, j][None, None, None, :]
    h = _layernorm(out, axis=-1)
    h = jnp.einsum('bhwc,ce->bhwe', h, w1) + b1
    h = _gelu(h)
    h = jnp.einsum('bhwe,ec->bhwc', h, w2) + b2
    return x + gamma[None, None, None, :] * h
```

```python
import functools
import math
import os

import jax
import jax.numpy as jnp
import numpy as np
from jax.experimental import pallas as pl
from jax.experimental.pallas import tpu as pltpu

_C1 = math.sqrt(2.0 / math.pi)
_C2 = _C1 * 0.044715
_S = _C2 ** (1.0 / 3.0)
_A = _C1 / _S

U = int("8")
ORDER = os.environ.get("K_ORDER", "")
ONEPASS = int(os.environ.get("K_ONEPASS", "1"))
XN_MODE = "bf16"
G_MODE = os.environ.get("K_G", "bbb")
PRE = int(os.environ.get("K_PRE", "2"))
MID = int(os.environ.get("K_MID", "5"))
MM2POS = "first"
NBI = 3
NBO = 3
LB = int(os.environ.get('K_LB', '1'))
LG = int("2")
LC = LB + LG
SX = 2 if LB == 1 else 4
SG = 2 if LG == 1 else 4
OFF = 2 + LC

f32 = jnp.float32
bf16 = jnp.bfloat16
u32 = jnp.uint32


def _kernel(x_hbm, dw_ref, w1_ref, b1_ref, w2t_ref, b2_ref, g_ref, o_hbm,
            xbuf, obuf, dwb, w1e, w2e, b2b, st1, st2, isem, osem, *rest, H, C, W, E):
    xs = rest[:U]
    XN = rest[U:U + SX]
    GS = [rest[U + SX + 3 * i:U + SX + 3 * i + 3] for i in range(SG)]
    NT = W // 128
    G = C // 8
    NCH = H // U
    NIT = -(-(H + OFF) // U)

    def in_copy(ch, slot):
        return pltpu.make_async_copy(x_hbm.at[pl.ds(ch * U, U)], xbuf.at[slot], isem.at[slot])

    def out_range(i):
        lo = max(U * i - OFF, 0)
        hi = min(U * i - OFF + U, H)
        return lo, hi

    full = [i for i in range(NIT) if out_range(i) == (U * i - OFF, U * i - OFF + U)]
    F0, F1 = full[0], full[-1] + 1

    def out_copy(i, slot):
        return pltpu.make_async_copy(obuf.at[slot], o_hbm.at[pl.ds(i * U - OFF, U)], osem.at[slot])

    def out_copy_static(i):
        lo, hi = out_range(i)
        if hi <= lo:
            return None
        k0 = lo - (U * i - OFF)
        return pltpu.make_async_copy(obuf.at[i % NBO, pl.ds(k0, hi - lo)], o_hbm.at[pl.ds(lo, hi - lo)], osem.at[i % NBO])

    in_copy(0, 0).start()
    in_copy(1, 1).start()

    for t in range(9):
        row = dw_ref[t // 3, pl.ds(t % 3, 1), :].astype(f32)
        row = jnp.concatenate([row, jnp.zeros((1, 128 - C), f32)], axis=1)
        sq = jnp.broadcast_to(row, (128, 128))
        dwb[t] = sq.T[:C, :]
    w1 = w1_ref[...].astype(f32)
    if ONEPASS:
        w1 = w1 - jnp.sum(w1, axis=0, keepdims=True) * (1.0 / C)
    b1 = b1_ref[...].astype(f32) * _S
    b1h = b1.astype(bf16).astype(f32)
    b1l = b1 - b1h
    rows = jax.lax.broadcasted_iota(jnp.int32, (128 - C, E), 0)
    ext = jnp.where(rows == 0, b1h, jnp.where(rows == 1, b1l, 0.0))
    w1full = jnp.concatenate([w1, ext], axis=0)
    w1e[...] = pltpu.bitcast(w1full.T.astype(bf16), u32)
    g = g_ref[...].astype(f32)
    gp = jnp.concatenate([g, jnp.zeros((1, 128 - C), f32)], axis=1)
    gcol = jnp.broadcast_to(gp, (128, 128)).T[:C, :]
    b2 = b2_ref[...].astype(f32) * g
    b2p = jnp.concatenate([b2, jnp.zeros((1, 128 - C), f32)], axis=1)
    b2b[...] = jnp.broadcast_to(b2p, (128, 128)).T[:C, :]
    w2t = w2t_ref[...].astype(f32)
    gfull = jnp.concatenate([gcol] * (E // 128), axis=1)
    w2e[...] = pltpu.bitcast((w2t * (gfull * (0.5 / _S))).astype(bf16), u32)
    prow = jax.lax.broadcasted_iota(jnp.int32, (128, W), 0)
    ones_rows = jnp.where((prow >= C) & (prow < C + 2), 1.0, 0.0).astype(f32)
    for s in range(SX):
        XN[s][...] = ones_rows if XN_MODE == "f32" else pltpu.bitcast(ones_rows.astype(bf16), u32)
    for s in range(SG):
        for e in range(3):
            GS[s][e][...] = jnp.zeros(GS[s][e].shape, GS[s][e].dtype)
    for s in range(U):
        xs[s][...] = jnp.zeros((C, W), f32)

    def tile(v):
        return jnp.concatenate([v] * NT, axis=1)

    def split(v):
        return [v[:, 128 * k:128 * (k + 1)] for k in range(NT)]

    class Row:
        pass

    def cvt(r, islot, k, g0, g1):
        cs = pl.ds(8 * g0, 8 * (g1 - g0))
        xs[r % U][cs, :] = xbuf[islot, k, cs, :].astype(f32)

    def conv_group(st, r, g):
        lane = jax.lax.broadcasted_iota(jnp.int32, (8, 128), 1)
        m0 = lane == 0
        m127 = lane == 127
        cs = pl.ds(8 * g, 8)
        x0 = xs[(r - 1) % U][cs, :]
        x1 = xs[r % U][cs, :]
        x2 = xs[(r + 1) % U][cs, :]
        t = []
        for j in range(3):
            t.append(tile(dwb[j, cs, :]) * x0 + tile(dwb[3 + j, cs, :]) * x1 + tile(dwb[6 + j, cs, :]) * x2)
        lt = [pltpu.roll(v, 1, 1) for v in split(t[0])]
        rt = [pltpu.roll(v, 127, 1) for v in split(t[2])]
        lft = [jnp.where(m0, 0.0 if k == 0 else lt[k - 1], lt[k]) for k in range(NT)]
        rgt = [jnp.where(m127, 0.0 if k == NT - 1 else rt[k + 1], rt[k]) for k in range(NT)]
        o = (jnp.concatenate(lft, axis=1) + t[1]) + jnp.concatenate(rgt, axis=1)
        if g == 0:
            st.outs = []
            st.s1 = o
            if ONEPASS:
                st.s2 = o * o
        else:
            st.s1 = st.s1 + o
            if ONEPASS:
                st.s2 = st.s2 + o * o
        st.outs.append(o)

    def bcast_rows(v):
        return jnp.concatenate([jnp.broadcast_to(v[k:k + 1, :], (8, 128)) for k in range(NT)], axis=1)

    def stats(st):
        if ONEPASS:
            for k, v in enumerate(split(st.s1) + split(st.s2)):
                st1[pl.ds(k, 8, stride=8), :] = v
            s = st1[pl.ds(0, 8), :]
            for j in range(1, 8):
                s = s + st1[pl.ds(8 * j, 8), :]
            s = s * (1.0 / C)
            var = pltpu.roll(s, 4, 0) - s * s
            rstd = jax.lax.rsqrt(jnp.maximum(var, 0.0) + 1e-5) * _S
            st.rstd = bcast_rows(rstd)
            st.ds = st.outs
        else:
            def allred(v, scr):
                for k, t in enumerate(split(v)):
                    scr[pl.ds(k, 8, stride=4), :] = t
                s = (scr[pl.ds(0, 8), :] + scr[pl.ds(8, 8), :]) + (scr[pl.ds(16, 8), :] + scr[pl.ds(24, 8), :])
                return s + pltpu.roll(s, 4, 0)
            m = bcast_rows(allred(st.s1, st1) * (1.0 / C))
            st.ds = [o - m for o in st.outs]
            sq = None
            for d in st.ds:
                sq = d * d if sq is None else sq + d * d
            v = allred(sq, st2) * (1.0 / C)
            st.rstd = bcast_rows(jax.lax.rsqrt(v + 1e-5) * _S)

    def normalize(st, r, to_scratch):
        xn = jnp.concatenate([d * st.rstd for d in st.ds], axis=0)
        if XN_MODE == "f32":
            XN[r % SX][pl.ds(0, C), :] = xn
        else:
            XN[r % SX][pl.ds(0, C // 2), :] = pltpu.bitcast(xn.astype(bf16), u32)

    def mm1(st, r):
        rhs = XN[r % SX][...]
        if XN_MODE != "f32":
            rhs = pltpu.bitcast(rhs, bf16)
        st.y = jnp.dot(pltpu.bitcast(w1e[...], bf16), rhs, preferred_element_type=f32)
        st.gl = []

    def gelu_chunk(st, j):
        y = st.y[16 * j:16 * (j + 1), :]
        u = y * (y * y + _A)
        st.gl.append(y * jnp.tanh(u) + y)

    def gelu_store(st, r, j):
        y = st.y[16 * j:16 * (j + 1), :]
        u = y * (y * y + _A)
        gl = y * jnp.tanh(u) + y
        e, jj = divmod(j, 8)
        if G_MODE[e] == "f":
            GS[r % SG][e][pl.ds(16 * jj, 16), :] = gl
        else:
            GS[r % SG][e][pl.ds(8 * jj, 8), :] = pltpu.bitcast(gl.astype(bf16), u32)

    def mm2_tile(st, r, e):
        gt = GS[r % SG][e][...]
        if G_MODE[e] != "f":
            gt = pltpu.bitcast(gt, bf16)
        w = pltpu.bitcast(w2e[:, pl.ds(128 * e, 128)], bf16)
        o = jnp.dot(w, gt, preferred_element_type=f32)
        st.acc = o if e == 0 else st.acc + o

    def mm2_lane(st, r, kk):
        acc = None
        ls = pl.ds(128 * kk, 128)
        for e in range(3):
            gt = GS[r % SG][e][:, ls]
            if G_MODE[e] != "f":
                gt = pltpu.bitcast(gt, bf16)
            w = pltpu.bitcast(w2e[:, pl.ds(128 * e, 128)], bf16)
            o = jnp.dot(w, gt, preferred_element_type=f32)
            acc = o if acc is None else acc + o
        if kk == 0:
            st.accs = []
        st.accs.append(acc + b2b[...] + xs[r % U][:, ls])

    def epi_pair(st, oslot, k, p):
        v = jnp.concatenate(st.accs[2 * p:2 * p + 2], axis=1)
        obuf[oslot, k, :, pl.ds(256 * p, 256)] = v.astype(bf16)

    def epilogue(st, r, oslot, k, g0, g1):
        cs = pl.ds(16 * g0, 16 * (g1 - g0))
        o = st.acc[16 * g0:16 * g1, :]
        obuf[oslot, k, cs, :] = (o + tile(b2b[cs, :]) + xs[r % U][cs, :]).astype(bf16)

    def body(i, islot, oslot):
        for k in range(U):
            r = k - 2
            A = Row()
            B = Row()
            Cc = Row()
            def do_mm2():
                for kk in range(4):
                    mm2_lane(Cc, r - LC, kk)
                    if kk % 2 == 1:
                        epi_pair(Cc, oslot, k, kk // 2)
            if MM2POS == "first":
                do_mm2()
            mm1(B, r - LB)
            if MM2POS == "after":
                do_mm2()
            for g in range(PRE):
                conv_group(A, r, g)
            g = PRE
            for j in range(24):
                gelu_store(B, r - LB, j)
                tgt = ((j + 1) * MID) // 24 + PRE
                while g < min(12, tgt):
                    conv_group(A, r, g)
                    g += 1
            if MM2POS == "late":
                do_mm2()
            while g < 12:
                conv_group(A, r, g)
                g += 1
            stats(A)
            cvt(r + 2, islot, k, 0, 12)
            normalize(A, r, True)

    def loop_body(i, _):
        islot = i % NBI
        oslot = i % NBO

        @pl.when(i < NCH)
        def _():
            in_copy(i, islot).wait()

        @pl.when(i >= NCH)
        def _():
            xbuf[islot] = jnp.zeros((U, C, W), bf16)

        @pl.when(i + 2 < NCH)
        def _():
            in_copy(i + 2, (i + 2) % NBI).start()

        @pl.when(i - NBO >= F0)
        def _():
            out_copy(i - NBO, oslot).wait()

        for ie in range(NIT):
            if ie not in full and ie - 0 + NBO < NIT and out_copy_static(ie) is not None:
                @pl.when(i == ie + NBO)
                def _(ie=ie):
                    out_copy_static(ie).wait()

        body(i, islot, oslot)

        @pl.when(jnp.logical_and(i >= F0, i < F1))
        def _():
            out_copy(i, oslot).start()

        for ie in range(NIT):
            if ie not in full and out_copy_static(ie) is not None:
                @pl.when(i == ie)
                def _(ie=ie):
                    out_copy_static(ie).start()
        return None

    jax.lax.fori_loop(0, NIT, loop_body, None)
    for i in range(NIT - NBO, NIT):
        if i in full:
            out_copy(i, i % NBO).wait()
        elif out_copy_static(i) is not None:
            out_copy_static(i).wait()


@jax.jit
def pallas_standalone__modern_conv_block_convnext__vision_kernel(x, dw, w1, b1, w2, b2, gamma):
    B, H, W, C = x.shape
    E = w1.shape[1]
    xt = jnp.transpose(x, (0, 1, 3, 2)).reshape(B * H, C, W)
    w2t = w2.T
    kern = functools.partial(_kernel, H=H, C=C, W=W, E=E)
    vm = pl.BlockSpec(memory_space=pltpu.VMEM)
    out = pl.pallas_call(
        kern,
        in_specs=[pl.BlockSpec(memory_space=pl.ANY), vm, vm, vm, vm, vm, vm],
        out_specs=pl.BlockSpec(memory_space=pl.ANY),
        out_shape=jax.ShapeDtypeStruct((H, C, W), x.dtype),
        scratch_shapes=[
            pltpu.VMEM((NBI, U, C, W), bf16),
            pltpu.VMEM((NBO, U, C, W), bf16),
            pltpu.VMEM((9, C, 128), f32),
            pltpu.VMEM((E // 2, 128), u32),
            pltpu.VMEM((C // 2, E), u32),
            pltpu.VMEM((C, 128), f32),
            pltpu.VMEM((64, 128), f32),
            pltpu.VMEM((64, 128), f32),
            pltpu.SemaphoreType.DMA((NBI,)),
            pltpu.SemaphoreType.DMA((NBO,)),
        ] + [pltpu.VMEM((C, W), f32)] * U
          + [pltpu.VMEM((128, W), f32) if XN_MODE == "f32" else pltpu.VMEM((64, W), u32)] * SX
          + [pltpu.VMEM((128, W), f32) if m == "f" else pltpu.VMEM((64, W), u32) for m in G_MODE] * SG,
        compiler_params=pltpu.CompilerParams(vmem_limit_bytes=100 * 1024 * 1024),
    )(xt, dw, w1, b1.reshape(1, E), w2t, b2.reshape(1, C), gamma.reshape(1, C))
    return jnp.transpose(out.reshape(B, H, C, W), (0, 1, 3, 2))
```

```python
import functools
import math
import os

import jax
import jax.numpy as jnp
import numpy as np
from jax.experimental import pallas as pl
from jax.experimental.pallas import tpu as pltpu

_C1 = math.sqrt(2.0 / math.pi)
_C2 = _C1 * 0.044715
_S = _C2 ** (1.0 / 3.0)
_A = _C1 / _S

U = int(os.environ.get("K_U", "8"))
ORDER = os.environ.get("K_ORDER", "")
ONEPASS = int(os.environ.get("K_ONEPASS", "1"))
XN_MODE = os.environ.get("K_XN", "bf16")
G_MODE = os.environ.get("K_G", "bbb")
PRE = int(os.environ.get("K_PRE", "2"))
MID = int(os.environ.get("K_MID", "5"))
STAGE_OUT = int(os.environ.get("K_SO", "1"))
def _prog(spec):
    out = []
    for tok in spec.split(","):
        if "-" in tok:
            t = tok[0]
            lo, hi = tok[1:].split("-")
            out += [t + str(j) for j in range(int(lo), int(hi) + 1)]
        else:
            out.append(tok)
    return out
PROG = _prog(os.environ.get("K_PROG", "m0-3,M,c0-11,g0-23,s,v,n"))
ASSOC = os.environ.get("K_ASSOC", "0")
NSUM = int(os.environ.get("K_NSUM", "12"))
DS2 = int(os.environ.get("K_DS2", "0"))
EPI = os.environ.get("K_EPI", "1")
MM2POS = os.environ.get("K_MM2", "after")
NBI = 3
NBO = 3
LB = int(os.environ.get('K_LB', '1'))
LG = int(os.environ.get('K_LG', '2'))
LC = LB + LG
SX = int(os.environ.get("K_SX", 4))
SG = int(os.environ.get("K_SG", 2 if LG == 1 else 4))
NO = int(os.environ.get("K_NO", "2"))
NS = int(os.environ.get("K_NS", "1"))
OFF = 2 + LC

f32 = jnp.float32
bf16 = jnp.bfloat16
u32 = jnp.uint32


def _kernel(x_hbm, dw_ref, w1_ref, b1_ref, w2t_ref, b2_ref, g_ref, o_hbm,
            xbuf, obuf, dwb, w1e, w2e, b2b, st1, st2, isem, osem, *rest, H, C, W, E):
    xs = rest[:U]
    XN = rest[U:U + SX]
    RT = rest[-2:]
    rest = rest[:-2]
    OUTS = rest[-NO - NS:-NS]
    ST = rest[-NS:]
    GS = [rest[U + SX + 3 * i:U + SX + 3 * i + 3] for i in range(SG)]
    NT = W // 128
    G = C // 8
    NCH = H // U
    NIT = -(-(H + OFF) // U)

    def in_copy(ch, slot):
        return pltpu.make_async_copy(x_hbm.at[pl.ds(ch * U, U)], xbuf.at[slot], isem.at[slot])

    def out_range(i):
        lo = max(U * i - OFF, 0)
        hi = min(U * i - OFF + U, H)
        return lo, hi

    full = [i for i in range(NIT) if out_range(i) == (U * i - OFF, U * i - OFF + U)]
    F0, F1 = full[0], full[-1] + 1

    def out_copy(i, slot):
        return pltpu.make_async_copy(obuf.at[slot], o_hbm.at[pl.ds(i * U - OFF, U)], osem.at[slot])

    def out_copy_static(i):
        lo, hi = out_range(i)
        if hi <= lo:
            return None
        k0 = lo - (U * i - OFF)
        return pltpu.make_async_copy(obuf.at[i % NBO, pl.ds(k0, hi - lo)], o_hbm.at[pl.ds(lo, hi - lo)], osem.at[i % NBO])

    in_copy(0, 0).start()
    in_copy(1, 1).start()

    for t in range(9):
        row = dw_ref[t // 3, pl.ds(t % 3, 1), :].astype(f32)
        row = jnp.concatenate([row, jnp.zeros((1, 128 - C), f32)], axis=1)
        sq = jnp.broadcast_to(row, (128, 128))
        dwb[t] = sq.T[:C, :]
    w1 = w1_ref[...].astype(f32)
    if ONEPASS:
        w1 = w1 - jnp.sum(w1, axis=0, keepdims=True) * (1.0 / C)
    b1 = b1_ref[...].astype(f32) * _S
    b1h = b1.astype(bf16).astype(f32)
    b1l = b1 - b1h
    rows = jax.lax.broadcasted_iota(jnp.int32, (128 - C, E), 0)
    ext = jnp.where(rows == 0, b1h, jnp.where(rows == 1, b1l, 0.0))
    w1full = jnp.concatenate([w1, ext], axis=0)
    w1e[...] = pltpu.bitcast(w1full.T.astype(bf16), u32)
    g = g_ref[...].astype(f32)
    gp = jnp.concatenate([g, jnp.zeros((1, 128 - C), f32)], axis=1)
    gcol = jnp.broadcast_to(gp, (128, 128)).T[:C, :]
    b2 = b2_ref[...].astype(f32) * g
    b2p = jnp.concatenate([b2, jnp.zeros((1, 128 - C), f32)], axis=1)
    b2b[...] = jnp.broadcast_to(b2p, (128, 128)).T[:C, :]
    w2t = w2t_ref[...].astype(f32)
    gfull = jnp.concatenate([gcol] * (E // 128), axis=1)
    w2e[...] = pltpu.bitcast((w2t * (gfull * (0.5 / _S))).astype(bf16), u32)
    prow = jax.lax.broadcasted_iota(jnp.int32, (128, W), 0)
    ones_rows = jnp.where((prow >= C) & (prow < C + 2), 1.0, 0.0).astype(f32)
    for s in range(SX):
        XN[s][...] = ones_rows if XN_MODE == "f32" else pltpu.bitcast(ones_rows.astype(bf16), u32)
    for s in range(SG):
        for e in range(3):
            GS[s][e][...] = jnp.zeros(GS[s][e].shape, GS[s][e].dtype)
    for s in range(U):
        xs[s][...] = jnp.zeros((C, W), f32)

    def tile(v):
        return jnp.concatenate([v] * NT, axis=1)

    def split(v):
        return [v[:, 128 * k:128 * (k + 1)] for k in range(NT)]

    class Row:
        pass

    def cvt(r, islot, k, g0, g1):
        cs = pl.ds(8 * g0, 8 * (g1 - g0))
        xs[r % U][cs, :] = xbuf[islot, k, cs, :].astype(f32)

    def conv_group(st, r, g):
        lane = jax.lax.broadcasted_iota(jnp.int32, (8, 128), 1)
        m0 = lane == 0
        m127 = lane == 127
        cs = pl.ds(8 * g, 8)
        x0 = xs[(r - 1) % U][cs, :]
        x1 = xs[r % U][cs, :]
        x2 = xs[(r + 1) % U][cs, :]
        t = []
        for j in range(3):
            t.append(tile(dwb[j, cs, :]) * x0 + tile(dwb[3 + j, cs, :]) * x1 + tile(dwb[6 + j, cs, :]) * x2)
        if os.environ.get("X_ROT2") == "1":
            lt = split(t[0])
        else:
            lt = [pltpu.roll(v, 1, 1) for v in split(t[0])]
        if os.environ.get("X_ROT") == "1":
            rt = split(t[2])
        else:
            rt = [pltpu.roll(v, 127, 1) for v in split(t[2])]
        lft = [jnp.where(m0, 0.0 if k == 0 else lt[k - 1], lt[k]) for k in range(NT)]
        rgt = [jnp.where(m127, 0.0 if k == NT - 1 else rt[k + 1], rt[k]) for k in range(NT)]
        lf, rg = jnp.concatenate(lft, axis=1), jnp.concatenate(rgt, axis=1)
        o = {"0": lambda: (lf + t[1]) + rg, "1": lambda: (lf + rg) + t[1], "2": lambda: (rg + t[1]) + lf}[ASSOC]()
        if g == 0:
            st.outs = []
            st.s1 = None
            st.s2 = None
        if g < NSUM:
            acc_sums(st, o)
        if STAGE_OUT:
            OUTS[r % NO][cs, :] = o
        else:
            st.outs.append(o)

    def acc_sums(st, o):
        st.s1 = o if st.s1 is None else st.s1 + o
        if DS2 == 0:
            st.s2 = o * o if st.s2 is None else st.s2 + o * o

    def bcast_rows(v):
        return jnp.concatenate([jnp.broadcast_to(v[k:k + 1, :], (8, 128)) for k in range(NT)], axis=1)

    def stats(st):
        st.ds = st.outs if not STAGE_OUT else [OUTS[st.r % NO][pl.ds(pl.multiple_of(st.z + 8 * g, 8), 8), :] for g in range(G)]
        ld2 = lambda g: OUTS[st.r % NO][pl.ds(pl.multiple_of(st.z2 + 8 * g, 8), 8), :]
        for g in range(NSUM, G):
            acc_sums(st, ld2(g))
        if DS2:
            for g in range(G):
                o = ld2(g)
                st.s2 = o * o if st.s2 is None else st.s2 + o * o
        if ONEPASS:
            for k, v in enumerate(split(st.s1) + split(st.s2)):
                ST[st.r % NS][pl.ds(k, 8, stride=8), :] = v
            s = ST[st.r % NS][pl.ds(0, 8), :]
            for j in range(1, 8):
                s = s + ST[st.r % NS][pl.ds(8 * j, 8), :]
            s = s * (1.0 / C)
            var = pltpu.roll(s, 4, 0) - s * s
            for q in range(int(os.environ.get("K_RT", "0"))):
                RT[st.r % 2][pl.ds(8 * q, 8), :] = var
                RT[st.r % 2][pl.ds(8 * q + 8, 8), :] = var
                var = RT[st.r % 2][pl.ds(8 * q + 4, 8), :]
            for q in range(int(os.environ.get("X_DLAT", "0"))):
                var = pltpu.roll(var, st.z, 1)
            for q in range(int(os.environ.get("X_LAT", "0"))):
                var = pltpu.roll(var, 1 if q % 2 == 0 else 127, 1)
            rstd = jax.lax.rsqrt(jnp.maximum(var, 0.0) + 1e-5) * _S if not os.environ.get("X_NOSQ") else var
            st.rstd = bcast_rows(rstd)
        else:
            def allred(v, scr):
                for k, t in enumerate(split(v)):
                    scr[pl.ds(k, 8, stride=4), :] = t
                s = (scr[pl.ds(0, 8), :] + scr[pl.ds(8, 8), :]) + (scr[pl.ds(16, 8), :] + scr[pl.ds(24, 8), :])
                return s + pltpu.roll(s, 4, 0)
            m = bcast_rows(allred(st.s1, st1) * (1.0 / C))
            st.ds = [o - m for o in st.outs]
            sq = None
            for d in st.ds:
                sq = d * d if sq is None else sq + d * d
            v = allred(sq, st2) * (1.0 / C)
            st.rstd = bcast_rows(jax.lax.rsqrt(v + 1e-5) * _S)

    def normalize(st, r, to_scratch):
        xn = jnp.concatenate([d * st.rstd for d in st.ds], axis=0)
        if XN_MODE == "f32":
            XN[r % SX][pl.ds(0, C), :] = xn
        else:
            XN[r % SX][pl.ds(0, C // 2), :] = pltpu.bitcast(xn.astype(bf16), u32)

    def mm1(st, r):
        rhs = XN[r % SX][...]
        if XN_MODE != "f32":
            rhs = pltpu.bitcast(rhs, bf16)
        st.y = jnp.dot(pltpu.bitcast(w1e[...], bf16), rhs, preferred_element_type=f32)
        st.gl = []

    def gelu_chunk(st, j):
        y = st.y[16 * j:16 * (j + 1), :]
        u = y * (y * y + _A)
        st.gl.append(y * jnp.tanh(u) + y)

    def mm1_part(st, r, e, n):
        rhs = XN[r % SX][...]
        if XN_MODE != "f32":
            rhs = pltpu.bitcast(rhs, bf16)
        rows = 192 // n
        w = pltpu.bitcast(w1e[pl.ds(rows * e, rows), :], bf16)
        if e == 0:
            st.y = []
            st.per = 24 // n
        st.y.append(jnp.dot(w, rhs, preferred_element_type=f32))

    def mm2_job(st, r, kk, e):
        ls = pl.ds(128 * kk, 128)
        if not hasattr(st, "accs"):
            st.accs = [None] * 4
        gt = GS[r % SG][e][:, ls]
        if G_MODE[e] != "f":
            gt = pltpu.bitcast(gt, bf16)
        w = pltpu.bitcast(w2e[:, pl.ds(128 * e, 128)], bf16)
        o = jnp.dot(w, gt, preferred_element_type=f32)
        st.accs[kk] = o if e == 0 else st.accs[kk] + o
        if e == 2:
            st.accs[kk] = st.accs[kk] + b2b[...] + xs[r % U][:, ls]

    def gelu_store(st, r, j):
        if isinstance(st.y, list):
            y = st.y[j // st.per][16 * (j % st.per):16 * (j % st.per + 1), :]
        else:
            y = st.y[16 * j:16 * (j + 1), :]
        if os.environ.get("X_CHEAP") == "1":
            gl = y * 1.5
        elif os.environ.get("X_CHEAP") == "2":
            gl = jnp.tanh(y) * y
        elif os.environ.get("X_CHEAP") == "5":
            u = y * (y * y + _A)
            gl = y * (u * 0.7 ) + y
        elif os.environ.get("X_CHEAP") == "6":
            u = y * (y * y + _A)
            gl = y * jnp.maximum(u, 0.7) + y
        elif os.environ.get("X_CHEAP") == "3":
            u = y * (y * y + _A)
            gl = y * jnp.tanh(u)
        elif os.environ.get("X_CHEAP") == "4":
            u = y * (y * y)
            gl = y * jnp.tanh(u)
        else:
            u = y * (y * y + _A)
            gl = y * jnp.tanh(u) + y
        e, jj = divmod(j, 8)
        if G_MODE[e] == "f":
            GS[r % SG][e][pl.ds(16 * jj, 16), :] = gl
        else:
            GS[r % SG][e][pl.ds(8 * jj, 8), :] = pltpu.bitcast(gl.astype(bf16), u32)

    def mm2_tile(st, r, e):
        gt = GS[r % SG][e][...]
        if G_MODE[e] != "f":
            gt = pltpu.bitcast(gt, bf16)
        w = pltpu.bitcast(w2e[:, pl.ds(128 * e, 128)], bf16)
        o = jnp.dot(w, gt, preferred_element_type=f32)
        st.acc = o if e == 0 else st.acc + o

    def mm2_lane(st, r, kk):
        acc = None
        ls = pl.ds(128 * kk, 128)
        for e in range(3):
            gt = GS[r % SG][e][:, ls]
            if G_MODE[e] != "f":
                gt = pltpu.bitcast(gt, bf16)
            w = pltpu.bitcast(w2e[:, pl.ds(128 * e, 128)], bf16)
            o = jnp.dot(w, gt, preferred_element_type=f32)
            acc = o if acc is None else acc + o
        if kk == 0:
            st.accs = []
        if EPI == "0":
            st.accs.append(acc + b2b[...] + xs[r % U][:, ls])
        else:
            st.accs.append(acc + (b2b[...] + xs[r % U][:, ls]))

    def epi_pair(st, oslot, k, p):
        v = jnp.concatenate(st.accs[2 * p:2 * p + 2], axis=1)
        obuf[oslot, k, :, pl.ds(256 * p, 256)] = v.astype(bf16)

    def epilogue(st, r, oslot, k, g0, g1):
        cs = pl.ds(16 * g0, 16 * (g1 - g0))
        o = st.acc[16 * g0:16 * g1, :]
        obuf[oslot, k, cs, :] = (o + tile(b2b[cs, :]) + xs[r % U][cs, :]).astype(bf16)

    def body(i, islot, oslot):
        for k in range(U):
            r = k - 2
            A = Row()
            A.r = r
            A.z = (i >> 20) * 8
            A.z2 = (i >> 21) * 8
            B = Row()
            Cc = Row()
            for tok in PROG:
                t, a = tok[0], (int(tok[1:]) if len(tok) > 1 else None)
                if t == "c":
                    conv_group(A, r, a)
                elif t == "m":
                    mm2_lane(Cc, r - LC, a)
                    if a % 2 == 1:
                        epi_pair(Cc, oslot, k, a // 2)
                elif t == "M":
                    if a is None:
                        mm1(B, r - LB)
                    else:
                        mm1_part(B, r - LB, a % 10, a // 10)
                elif t == "j":
                    mm2_job(Cc, r - LC, a // 10 - 1, a % 10)
                    if a % 10 == 2 and (a // 10 - 1) % 2 == 1:
                        epi_pair(Cc, oslot, k, (a // 10 - 1) // 2)
                elif t == "g":
                    gelu_store(B, r - LB, a)
                elif t == "s":
                    stats(A)
                elif t == "v":
                    cvt(r + 2, islot, k, 0, 12)
                elif t == "w":
                    cvt(r + 2, islot, k, a, a + 1)
                elif t == "n":
                    normalize(A, r, True)

    def loop_body(i, _):
        islot = i % NBI
        oslot = i % NBO

        @pl.when(i < NCH)
        def _():
            in_copy(i, islot).wait()

        @pl.when(i >= NCH)
        def _():
            xbuf[islot] = jnp.zeros((U, C, W), bf16)

        @pl.when(i + 2 < NCH)
        def _():
            in_copy(i + 2, (i + 2) % NBI).start()

        @pl.when(i - NBO >= F0)
        def _():
            out_copy(i - NBO, oslot).wait()

        for ie in range(NIT):
            if ie not in full and ie - 0 + NBO < NIT and out_copy_static(ie) is not None:
                @pl.when(i == ie + NBO)
                def _(ie=ie):
                    out_copy_static(ie).wait()

        body(i, islot, oslot)

        @pl.when(jnp.logical_and(i >= F0, i < F1))
        def _():
            out_copy(i, oslot).start()

        for ie in range(NIT):
            if ie not in full and out_copy_static(ie) is not None:
                @pl.when(i == ie)
                def _(ie=ie):
                    out_copy_static(ie).start()
        return None

    jax.lax.fori_loop(0, NIT, loop_body, None)
    for i in range(NIT - NBO, NIT):
        if i in full:
            out_copy(i, i % NBO).wait()
        elif out_copy_static(i) is not None:
            out_copy_static(i).wait()


@jax.jit
def pallas_standalone__modern_conv_block_convnext__vision_kernel(x, dw, w1, b1, w2, b2, gamma):
    B, H, W, C = x.shape
    E = w1.shape[1]
    xt = jnp.transpose(x, (0, 1, 3, 2)).reshape(B * H, C, W)
    w2t = w2.T
    kern = functools.partial(_kernel, H=H, C=C, W=W, E=E)
    vm = pl.BlockSpec(memory_space=pltpu.VMEM)
    out = pl.pallas_call(
        kern,
        in_specs=[pl.BlockSpec(memory_space=pl.ANY), vm, vm, vm, vm, vm, vm],
        out_specs=pl.BlockSpec(memory_space=pl.ANY),
        out_shape=jax.ShapeDtypeStruct((H, C, W), x.dtype),
        scratch_shapes=[
            pltpu.VMEM((NBI, U, C, W), bf16),
            pltpu.VMEM((NBO, U, C, W), bf16),
            pltpu.VMEM((9, C, 128), f32),
            pltpu.VMEM((E // 2, 128), u32),
            pltpu.VMEM((C // 2, E), u32),
            pltpu.VMEM((C, 128), f32),
            pltpu.VMEM((64, 128), f32),
            pltpu.VMEM((64, 128), f32),
            pltpu.SemaphoreType.DMA((NBI,)),
            pltpu.SemaphoreType.DMA((NBO,)),
        ] + [pltpu.VMEM((C, W), f32)] * U
          + [pltpu.VMEM((128, W), f32) if XN_MODE == "f32" else pltpu.VMEM((64, W), u32)] * SX
          + [pltpu.VMEM((128, W), f32) if m == "f" else pltpu.VMEM((64, W), u32) for m in G_MODE] * SG + [pltpu.VMEM((C, W), f32)] * NO + [pltpu.VMEM((64, 128), f32)] * NS + [pltpu.VMEM((520, 128), f32)] * 2,
        compiler_params=pltpu.CompilerParams(vmem_limit_bytes=100 * 1024 * 1024,
            flags={f: True for f in os.environ.get("K_FLAGS", "").split(",") if f} or None),
    )(xt, dw, w1, b1.reshape(1, E), w2t, b2.reshape(1, C), gamma.reshape(1, C))
    return jnp.transpose(out.reshape(B, H, C, W), (0, 1, 3, 2))
```

```python
import functools
import math

import jax
import jax.numpy as jnp
import numpy as np
from jax.experimental import pallas as pl
from jax.experimental.pallas import tpu as pltpu

_C1 = math.sqrt(2.0 / math.pi)
_C2 = _C1 * 0.044715
_S = _C2 ** (1.0 / 3.0)
_A = _C1 / _S


def _env(name, default):
    return default


def _prog(spec):
    out = []
    for tok in spec.split(","):
        if "-" in tok:
            t = tok[0]
            lo, hi = tok[1:].split("-")
            out += [t + str(j) for j in range(int(lo), int(hi) + 1)]
        else:
            out.append(tok)
    return out


U = int(_env("K_U", "16"))
MODE = _env("K_MODE", "V")
PROG = _prog(_env("K_PROG", "m0-3,M,c0-11,g0-23,s,v,n"))
NBI = 4
NBO = 4
LR = int(_env("K_LR", "1"))
LA = (LR + 2) if MODE == "H" else 2
LB = int(_env("K_LB", "1"))
LG = int(_env("K_LG", "2"))
SX = int(_env("K_SX", "4"))
SG = int(_env("K_SG", "2"))
SH = int(_env("K_SH", "4"))
NO = int(_env("K_NO", "2"))
OFF = LA + LB + LG
BARR = _env("K_BARR", "g")

DEFER = int(_env("K_DEFER", "1"))
f32 = jnp.float32
bf16 = jnp.bfloat16
u32 = jnp.uint32


def _kernel(x_hbm, dw_ref, w1_ref, b1_ref, w2t_ref, b2_ref, g_ref, o_hbm,
            xbuf, obuf, dwb, w1e, w2e, b2b, ST, isem, osem, *rest, H, C, W, E):
    rest = list(rest)
    MAN = _env("K_MAN", "1") == "1"
    if MAN:
        wsem = rest.pop()
        src = [dw_ref, w1_ref, b1_ref, w2t_ref, b2_ref, g_ref]
        dst = rest[-6:]
        del rest[-6:]
        wcopies = [pltpu.make_async_copy(a, b, wsem.at[j]) for j, (a, b) in enumerate(zip(src, dst))]
        dw_ref, w1_ref, b1_ref, w2t_ref, b2_ref, g_ref = dst

    def take(n):
        out = rest[:n]
        del rest[:n]
        return out

    def rot(l, name):
        n = int(_env("R_" + name, {"X": 3, "N": 3, "G": 1, "O": 1}.get(name, 0))) % len(l)
        return l[n:] + l[:n]

    xs = rot(take(U), "X")
    XN = rot(take(SX), "N")
    GS = rot([take(3) for _ in range(SG)], "G")
    OUTS = rot(take(NO), "O")
    OUTT = None
    XL = rot(take(SH), "H")
    XR = rot(take(SH), "H")
    NT = W // 128
    G = C // 8
    NIT = int(_env("X_IT", H // U))

    NI = int(_env("K_NI", "1"))
    UI = U // NI

    class in_copy:
        def __init__(self, ch):
            self.ch = ch

        def part(self, q):
            start = jnp.minimum(OFF + self.ch * U, H - U)
            slot = self.ch % NBI
            if "i" in _env("X_NODMA", ""):
                return pltpu.make_async_copy(x_hbm.at[pl.ds(start + q * UI, 1)], xbuf.at[slot, pl.ds(q * UI, 1)], isem.at[slot, q])
            return pltpu.make_async_copy(x_hbm.at[pl.ds(start + q * UI, UI)], xbuf.at[slot, pl.ds(q * UI, UI)], isem.at[slot, q])

        def start(self):
            for q in range(NI):
                self.part(q).start()

        def wait(self):
            for q in range(NI):
                self.part(q).wait()

    def head_copy():
        return pltpu.make_async_copy(x_hbm.at[pl.ds(0, OFF)], xbuf.at[NBI - 1, pl.ds(0, OFF)], isem.at[NBI - 1, 0])

    NP = int(_env("K_NP", "4"))
    UP = U // NP

    class out_copy:
        def __init__(self, i):
            self.i = i

        def part(self, q):
            slot = self.i % NBO
            if "o" in _env("X_NODMA", ""):
                return pltpu.make_async_copy(obuf.at[slot, pl.ds(q * UP, 1)], o_hbm.at[pl.ds(self.i * U + q * UP, 1)], osem.at[slot, q])
            return pltpu.make_async_copy(obuf.at[slot, pl.ds(q * UP, UP)], o_hbm.at[pl.ds(self.i * U + q * UP, UP)], osem.at[slot, q])

        def start(self):
            self.part(NP - 1).start()

        def wait(self):
            for q in range(NP):
                self.part(q).wait()

    if MAN:
        for cp in wcopies:
            cp.start()
    head_copy().start()
    in_copy(0).start()
    if _env("K_D1", "1") == "0":
        in_copy(1).start()

    def column(row):
        row = jnp.concatenate([row, jnp.zeros((1, 128 - C), f32)], axis=1)
        return jnp.broadcast_to(row, (128, 128)).T[:C, :]

    def prepare():
        if MAN:
            for cp in wcopies:
                cp.wait()
        for t in range(9):
            dwb[t] = column(dw_ref[t // 3, pl.ds(t % 3, 1), :].astype(f32))
        w1 = w1_ref[...].astype(f32)
        w1 = w1 - jnp.sum(w1, axis=0, keepdims=True) * (1.0 / C)
        b1 = b1_ref[...].astype(f32) * _S
        b1h = b1.astype(bf16).astype(f32)
        b1l = b1 - b1h
        rows = jax.lax.broadcasted_iota(jnp.int32, (128 - C, E), 0)
        ext = jnp.where(rows == 0, b1h, jnp.where(rows == 1, b1l, 0.0))
        w1full = jnp.concatenate([w1, ext], axis=0)
        w1e[...] = pltpu.bitcast(w1full.T.astype(bf16), u32)
        g = g_ref[...].astype(f32)
        gcol = column(g)
        b2b[...] = column(b2_ref[...].astype(f32) * g)
        w2t = w2t_ref[...].astype(f32)
        gfull = jnp.concatenate([gcol] * (E // 128), axis=1)
        w2e[...] = pltpu.bitcast((w2t * (gfull * (0.5 / _S))).astype(bf16), u32)
        prow = jax.lax.broadcasted_iota(jnp.int32, (128 - C, W), 0)
        ones_rows = pltpu.bitcast(jnp.where(prow < 2, 1.0, 0.0).astype(bf16), u32)
        for s in range(SX):
            XN[s][pl.ds(C // 2, 64 - C // 2), :] = ones_rows
        for ref in xs + XL + XR + XN + OUTS + sum(GS, []):
            ref[pl.ds(0, 8), pl.ds(0, 128)] = jnp.zeros((8, 128), ref.dtype)
        xs[-1 % U][...] = jnp.zeros((C, W), f32)
        if MODE == "H":
            XL[-1 % SH][...] = jnp.zeros((C, W), f32)
            XR[-1 % SH][...] = jnp.zeros((C, W), f32)
        xbuf[(NIT - 1) % NBI, U] = jnp.zeros((C, W), bf16)

        return b1l

    def tile(v):
        return jnp.concatenate([v] * NT, axis=1)

    def split(v):
        return [v[:, 128 * k:128 * (k + 1)] for k in range(NT)]

    class Row:
        pass

    DZ = _env("K_DZ", "")

    def dz(name, z, off, n):
        return pl.ds(pl.multiple_of(z + off, 8), n) if name in DZ else pl.ds(off, n)

    def cvt(r, islot, k, z):
        xs[r % U][dz("x", z, 0, C), :] = xbuf[islot, k].astype(f32)

    def shift_group(r, g, z):
        lane = jax.lax.broadcasted_iota(jnp.int32, (8, 128), 1)
        cs = dz("h", z, 8 * g, 8)
        x = split(xs[r % U][pl.ds(pl.multiple_of(z + 8 * g, 8), 8), :])
        for k in range(NT):
            lt = pltpu.roll(x[k], 1, 1)
            if k == 0:
                pltpu.store(XL[r % SH].at[cs, pl.ds(0, 128)], jnp.where(lane != 0, lt, 0.0))
            else:
                XL[r % SH][cs, pl.ds(128 * k, 128)] = lt
            if k < NT - 1:
                pltpu.store(XL[r % SH].at[cs, pl.ds(128 * k + 128, 128)], lt, mask=lane == 0)
        for k in reversed(range(NT)):
            rt = pltpu.roll(x[k], 127, 1)
            if k == NT - 1:
                pltpu.store(XR[r % SH].at[cs, pl.ds(128 * k, 128)], jnp.where(lane != 127, rt, 0.0))
            else:
                XR[r % SH][cs, pl.ds(128 * k, 128)] = rt
            if k > 0:
                pltpu.store(XR[r % SH].at[cs, pl.ds(128 * k - 128, 128)], rt, mask=lane == 127)

    def conv_group(st, g):
        r = st.r
        cs = pl.ds(8 * g, 8)
        if MODE == "V":
            lane = jax.lax.broadcasted_iota(jnp.int32, (8, 128), 1)
            m0 = lane == 0
            m127 = lane == 127
            x0 = xs[(r - 1) % U][cs, :]
            x1 = xs[r % U][cs, :]
            x2 = xs[(r + 1) % U][cs, :]
            t = []
            for j in range(3):
                t.append(tile(dwb[j, cs, :]) * x0 + tile(dwb[3 + j, cs, :]) * x1 + tile(dwb[6 + j, cs, :]) * x2)
            lt = [pltpu.roll(v, 1, 1) for v in split(t[0])]
            rt = [pltpu.roll(v, 127, 1) for v in split(t[2])]
            lft = [jnp.where(m0, 0.0 if k == 0 else lt[k - 1], lt[k]) for k in range(NT)]
            rgt = [jnp.where(m127, 0.0 if k == NT - 1 else rt[k + 1], rt[k]) for k in range(NT)]
            lf, rg = jnp.concatenate(lft, axis=1), jnp.concatenate(rgt, axis=1)
            o = (lf + t[1]) + rg
        else:
            t = []
            for i in range(3):
                q = r + i - 1
                t.append(tile(dwb[3 * i, cs, :]) * XL[q % SH][cs, :] + tile(dwb[3 * i + 1, cs, :]) * xs[q % U][cs, :]
                         + tile(dwb[3 * i + 2, cs, :]) * XR[q % SH][cs, :])
            o = (t[0] + t[1]) + t[2]
        GA = int(_env("K_GA", "0"))
        for q in range(int(_env("K_SRT", "0")) if g > 0 else 0):
            SR[q, cs, :] = st.s1
            st.s1 = SR[q, pl.ds(pl.multiple_of(st.z + 8 * g, 8), 8), :]
        if g == GA and GA:
            st.a = split(st.s1) + split(st.s2)
            for q in range(int(_env("K_DA", "0"))):
                st.a = [pltpu.roll(v, st.z, 1) for v in st.a]
            if _env("K_AM", "0") == "0":
                st.s1 = jnp.concatenate(st.a[:NT], axis=1) + o
                st.s2 = jnp.concatenate(st.a[NT:], axis=1) + o * o
            else:
                st.sa1 = jnp.concatenate(st.a[:NT], axis=1)
                st.sa2 = jnp.concatenate(st.a[NT:], axis=1)
                st.s1 = o
                st.s2 = o * o
        elif g == 0:
            st.s1 = o
            st.s2 = o * o
        else:
            st.s1 = st.s1 + o
            st.s2 = st.s2 + o * o
        if g == G - 1 and GA and _env("K_AM", "0") != "0":
            st.s1 = st.s1 + st.sa1
            st.s2 = st.s2 + st.sa2
        OUTS[r % NO][cs, :] = o

    def bcast_rows(v):
        return jnp.concatenate([jnp.broadcast_to(v[k:k + 1, :], (8, 128)) for k in range(NT)], axis=1)

    def stats(st):
        stats_a(st)
        stats_b(st)

    def stats_a(st):
        for k, v in enumerate(split(st.s1) + split(st.s2)):
            ST[pl.ds(k, 8, stride=8), :] = v

    def stats_b(st):
        st.ds = [OUTS[st.r % NO][pl.ds(pl.multiple_of(st.z + 8 * g, 8), 8), :] for g in range(G)]
        s = ST[pl.ds(0, 8), :]
        for j in range(1, 8):
            s = s + ST[pl.ds(8 * j, 8), :]
        s = s * (1.0 / C)
        var = pltpu.roll(s, 4, 0) - s * s
        for q in range(int(_env("K_DLAT", "0"))):
            var = pltpu.roll(var, st.z, 1)
        ve = jnp.maximum(var, 0.0) + 1e-5
        rs = jax.lax.rsqrt(ve)
        st.mk2 = s
        MK = _env("K_MK", "")
        st.mk = {"": None, "v": ve, "r": rs, "s": s}[MK]
        st.rstd = bcast_rows(rs * _S)

    def normalize(st):
        ds = st.ds
        if (st.mk is not None and str(st.r % U) not in _env('K_MKX', '')) or _env("K_OD", "0") == "1":
            O = OUTT[st.r % NO]
            if st.mk is not None:
                O[1, pl.ds(0, 8), pl.ds(0, 128)] = st.mk
            n0 = int(_env("K_MK0", "0"))
            ds = ds[:n0] + [O[st.z, pl.ds(8 * g, 8), :] for g in range(n0, G)]
        xn = jnp.concatenate([d * st.rstd for d in ds], axis=0)
        pk = pltpu.bitcast(xn.astype(bf16), u32)
        XN[st.r % SX][dz('n', st.z, 0, C // 2), :] = pk
        if str(st.k) in _env("K_PRI", "-"):
            for q in range(int(_env("K_PN", "1"))):
                v = (pk[C // 2 - 8:, :128] if _env("K_PW", "n") == "n" else st.mk2) if q == 0 else v
                v = pltpu.roll(v, 1, 1)
            SR[0, pl.ds(0, 8), pl.ds(0, 128)] += v if v.dtype == f32 else pltpu.bitcast(v, f32)

    def mm1(st, r):
        rhs = pltpu.bitcast(XN[r % SX][...], bf16)
        st.y = jnp.dot(pltpu.bitcast(w1e[...], bf16), rhs, preferred_element_type=f32)

    def gelu_store(st, r, j, z):
        y = st.y[16 * j:16 * (j + 1), :]
        u = y * (y * y + _A)
        gl = y * jnp.tanh(u) + y
        e, jj = divmod(j, 8)
        GS[r % SG][e][dz('g', z, 8 * jj, 8), :] = pltpu.bitcast(gl.astype(bf16), u32)

    def mm2_lane(st, r, kk):
        acc = None
        ls = pl.ds(128 * kk, 128)
        for e in range(3):
            gt = pltpu.bitcast(GS[r % SG][e][:, ls], bf16)
            w = pltpu.bitcast(w2e[:, pl.ds(128 * e, 128)], bf16)
            o = jnp.dot(w, gt, preferred_element_type=f32)
            acc = o if acc is None else acc + o
        if kk == 0:
            st.accs = []
        st.accs.append(acc + (b2b[...] + xs[r % U][:, ls]))

    def epi_pair(st, oslot, k, p):
        v = jnp.concatenate(st.accs[2 * p:2 * p + 2], axis=1)
        obuf[oslot, k, :, pl.ds(256 * p, 256)] = v.astype(bf16)

    def phase(p, k, islot, irow, oslot, z, lo=-10 ** 9, i=None):
        A = Row()
        A.r = p - LA
        A.z, A.k = z, k
        B = Row()
        Cc = Row()
        rb, rc = p - LA - LB, p - OFF
        defer = DEFER and (k == U - 1 or (k is None and p == OFF - 1))
        prog = PROG
        if DEFER and k == 0:
            ps = _prog(_env("K_PROG0", "N," + ",".join(PROG)))
            prog = ps
        for tok in prog:
            t, a = tok[0], (int(tok[1:]) if len(tok) > 1 else None)
            if t == "o" and i is not None and (k + 1) % UP == 0 and not (OH and k == U - 1):
                out_copy(i).part(k // UP).start()
            elif t == "i" and i is not None and k % UI == int(_env("K_LK", "2")):
                in_copy(i + 2).part(k // UI).start()
            elif t == "w" and i is not None and k % UI == 0:
                in_copy(i).part(k // UI).wait()
            elif t == "c" and A.r >= lo:
                conv_group(A, a)
            elif t == "s" and A.r >= lo:
                stats_a(A) if defer else stats(A)
            elif t == "n" and A.r >= lo:
                if not defer:
                    normalize(A)
            elif t == "N":
                D = Row()
                D.r, D.z, D.k = A.r - 1, z, None
                stats_b(D)
                normalize(D)
            elif t == "m" and rc >= lo:
                mm2_lane(Cc, rc, a)
                if a % 2 == 1:
                    epi_pair(Cc, oslot, k, a // 2)
            elif t == "M" and rb >= lo:
                mm1(B, rb)
            elif t == "g" and rb >= lo:
                gelu_store(B, rb, a, z)
            elif t == "r" and MODE == "H" and p - LR >= lo:
                shift_group(p - LR, a, z)
            elif t == "v":
                cvt(p, islot, irow, z)

    head_copy().wait()
    if _env("K_LATE", "2") == "1":
        in_copy(2).start()
    one = None
    del one

    LW = _env("K_LW", "")
    if "i" in LW:
        in_copy(0).wait()
    OH = int(_env("K_OH", "0"))
    WI = int(_env('K_WI', '0'))
    if _env("K_D1", "1") == "1":
        in_copy(1).start()
    NREP = int(_env("K_NREP", "1"))

    def loop_body(i0, _):
        for rep in range(NREP):
            i = i0 * NREP + rep
            islot = i % NBI
            oslot = i % NBO
            if OH:
                @pl.when(i >= 1)
                def _():
                    out_copy(i - 1).start()
            if "i" not in LW and not WI:
                in_copy(i).wait()
            if "b" in BARR:
                @pl.when(i > 1000)
                def _():
                    xbuf[islot] = jnp.zeros((U + 1, C, W), bf16)
            if _env("K_LATE", "2") == "0":
                in_copy(i + 2).start()

            if "o" not in LW:
                @pl.when(i >= NBO)
                def _():
                    out_copy(i - NBO).wait()

            z = (i >> 21) * 8
            delta = jnp.maximum(OFF + i * U - (H - U), 0)
            for k in range(U):
                if WI and k % UI == 0 and _env("K_WP", "0") == "0":
                    in_copy(i).part(k // UI).wait()
                phase(OFF + k, k, islot, jnp.minimum(k + delta, U), oslot, z, i=i)
                if (k + 1) % UP == 0 and k + 1 < U and 'o' not in PROG:
                    out_copy(i).part(k // UP).start()
                if _env("K_LATE", "2") == "2" and k % UI == int(_env("K_LK", "2")):
                    in_copy(i + 2).part(k // UI).start()
            if 'o' not in PROG and not OH:
                out_copy(i).start()
            if _env("K_LATE", "2") == "1":
                in_copy(i + 3).start()
            if "i" in LW:
                in_copy(i + 1).wait()
            if "o" in LW:
                @pl.when(i + 1 >= NBO)
                def _():
                    out_copy(i + 1 - NBO).wait()
        return None

    def fill(i):
        z = (i >> 21) * 8
        for p in range(OFF):
            phase(p, None, NBI - 1, p, None, z, lo=0)
        return None

    if "g" in BARR:
        pid = pl.program_id(0)
    elif "d" in BARR:
        bits = pltpu.bitcast(dw_ref[0, pl.ds(0, 2), :].astype(f32), jnp.int32)
        pid = (jnp.max(bits) & 1) >> 1
    else:
        b1l = prepare()
        bits = pltpu.bitcast(b1l[:, :128], jnp.int32)
        pid = jnp.max(bits & 1) >> 1

    @pl.when(pid == 0)
    def _():
        if "g" in BARR or "d" in BARR:
            prepare()
        fill(pid)
    jax.lax.fori_loop(0, NIT // NREP, loop_body, None)
    if _env("K_PRI", "-") != "-":
        @pl.when(jnp.max(pltpu.bitcast(SR[0, pl.ds(0, 8), pl.ds(0, 128)], jnp.int32) & 1) > 1)
        def _():
            xbuf[0, 0] = jnp.zeros((C, W), bf16)
    if OH:
        out_copy(NIT - 1).start()
    if "i" not in LW:
        in_copy(NIT).wait()
    in_copy(NIT + 1).wait()
    if _env("K_LATE", "2") == "1":
        in_copy(NIT + 2).wait()
    for i in range(NIT - NBO + ("o" in LW), NIT):
        out_copy(i).wait()


def isem_one(r):
    return 0


@jax.jit
def pallas_standalone__modern_conv_block_convnext__vision_kernel(x, dw, w1, b1, w2, b2, gamma):
    B, H, W, C = x.shape
    E = w1.shape[1]
    xt = jnp.transpose(x, (0, 1, 3, 2)).reshape(B * H, C, W)
    w2t = w2.T
    kern = functools.partial(_kernel, H=H, C=C, W=W, E=E)
    man = _env("K_MAN", "1") == "1"
    ws = (dw, w1, b1.reshape(1, E), w2t, b2.reshape(1, C), gamma.reshape(1, C))
    vm = pl.BlockSpec(memory_space=pltpu.VMEM) if _env('K_VM', '1') == '1' else None
    out = pl.pallas_call(
        kern,
        grid=(1,),
        in_specs=[pl.BlockSpec(memory_space=pl.ANY), vm, vm, vm, vm, vm, vm] if not man else [pl.BlockSpec(memory_space=pl.ANY)] * 7,
        out_specs=pl.BlockSpec(memory_space=pl.ANY),
        out_shape=jax.ShapeDtypeStruct((H, C, W), x.dtype),
        scratch_shapes=[
            pltpu.VMEM((NBI, U + 1, C, W), bf16),
            pltpu.VMEM((NBO, U, C, W), bf16),
            pltpu.VMEM((9, C, 128), f32),
            pltpu.VMEM((E // 2, 128), u32),
            pltpu.VMEM((C // 2, E), u32),
            pltpu.VMEM((C, 128), f32),
            pltpu.VMEM((64, 128), f32),
            pltpu.SemaphoreType.DMA((NBI, int(_env('K_NI', '1')))),
            pltpu.SemaphoreType.DMA((NBO, int(_env("K_NP", "4")))),
        ] + [pltpu.VMEM((C, W), f32)] * U
          + [pltpu.VMEM((64, W), u32)] * SX
          + [pltpu.VMEM((64, W), u32)] * (3 * SG)
          + [pltpu.VMEM((C, W), f32)] * NO
          + [pltpu.VMEM((C, W), f32)] * (2 * SH)
          + ([pltpu.VMEM(w.shape, w.dtype) for w in ws] + [pltpu.SemaphoreType.DMA((6,))] if man else []),
        compiler_params=pltpu.CompilerParams(vmem_limit_bytes=100 * 1024 * 1024, disable_bounds_checks=bool(int(_env("K_DBC", "1")))),
    )(xt, *ws)
    return jnp.transpose(out.reshape(B, H, C, W), (0, 1, 3, 2))
```

```python
import functools
import math

import jax
import jax.numpy as jnp
import numpy as np
from jax.experimental import pallas as pl
from jax.experimental.pallas import tpu as pltpu

_C1 = math.sqrt(2.0 / math.pi)
_C2 = _C1 * 0.044715
_S = _C2 ** (1.0 / 3.0)
_A = _C1 / _S


def _env(name, default):
    return default


def _prog(spec):
    out = []
    for tok in spec.split(","):
        if "-" in tok:
            t = tok[0]
            lo, hi = tok[1:].split("-")
            out += [t + str(j) for j in range(int(lo), int(hi) + 1)]
        else:
            out.append(tok)
    return out


U = int(_env("K_U", "32"))
MODE = _env("K_MODE", "V")
PROG = _prog(_env("K_PROG", "v,c0-11,s,n,m0-3,M,g0-23,o"))
NBI = 4
NBO = 4
LR = int(_env("K_LR", "1"))
LA = (LR + 2) if MODE == "H" else 2
LB = int(_env("K_LB", "1"))
LG = int(_env("K_LG", "3"))
SX = int(_env("K_SX", "2"))
SG = int(_env("K_SG", "4"))
SH = int(_env("K_SH", "4"))
NO = int(_env("K_NO", "2"))
OFF = LA + LB + LG
BARR = _env("K_BARR", "g")

GM = _env("K_G", "bbb")
XM = _env('K_XM', 'b')
DEFER = int(_env("K_DEFER", "1"))
f32 = jnp.float32
bf16 = jnp.bfloat16
u32 = jnp.uint32


def _kernel(x_hbm, dw_ref, w1_ref, b1_ref, w2t_ref, b2_ref, g_ref, o_hbm,
            xbuf, obuf, dwb, w1e, w2e, b2b, ST, isem, osem, *rest, H, C, W, E):
    rest = list(rest)
    MAN = _env("K_MAN", "1") == "1"
    if MAN:
        wsem = rest.pop()
        src = [dw_ref, w1_ref, b1_ref, w2t_ref, b2_ref, g_ref]
        dst = rest[-6:]
        del rest[-6:]
        wcopies = [pltpu.make_async_copy(a, b, wsem.at[j]) for j, (a, b) in enumerate(zip(src, dst))]
        dw_ref, w1_ref, b1_ref, w2t_ref, b2_ref, g_ref = dst

    def take(n):
        out = rest[:n]
        del rest[:n]
        return out

    def rot(l, name):
        n = int(_env("R_" + name, {"X": 3, "N": 3, "G": 1, "O": 1}.get(name, 0))) % len(l)
        return l[n:] + l[:n]

    xs = rot(take(U), "X")
    XN = rot(take(SX), "N")
    GS = rot([take(3) for _ in range(SG)], "G")
    OUTS = rot(take(NO), "O")
    OUTT = None
    XL = rot(take(SH), "H")
    XR = rot(take(SH), "H")
    RT = take(8)
    NT = W // 128
    G = C // 8
    NIT = int(_env("X_IT", H // U))

    NI = int(_env("K_NI", "2"))
    UI = U // NI

    class in_copy:
        def __init__(self, ch):
            self.ch = ch

        def part(self, q):
            start = jnp.minimum(OFF + self.ch * U, H - U)
            slot = self.ch % NBI
            if "i" in _env("X_NODMA", ""):
                return pltpu.make_async_copy(x_hbm.at[pl.ds(start + q * UI, 1)], xbuf.at[slot, pl.ds(q * UI, 1)], isem.at[slot, q])
            return pltpu.make_async_copy(x_hbm.at[pl.ds(start + q * UI, UI)], xbuf.at[slot, pl.ds(q * UI, UI)], isem.at[slot, q])

        def start(self):
            for q in range(NI):
                self.part(q).start()

        def wait(self):
            for q in range(NI):
                self.part(q).wait()

    def head_copy():
        return pltpu.make_async_copy(x_hbm.at[pl.ds(0, OFF)], xbuf.at[NBI - 1, pl.ds(0, OFF)], isem.at[NBI - 1, 0])

    NP = int(_env("K_NP", "4"))
    UP = U // NP

    class out_copy:
        def __init__(self, i):
            self.i = i

        def part(self, q):
            slot = self.i % NBO
            if "o" in _env("X_NODMA", ""):
                return pltpu.make_async_copy(obuf.at[slot, pl.ds(q * UP, 1)], o_hbm.at[pl.ds(self.i * U + q * UP, 1)], osem.at[slot, q])
            return pltpu.make_async_copy(obuf.at[slot, pl.ds(q * UP, UP)], o_hbm.at[pl.ds(self.i * U + q * UP, UP)], osem.at[slot, q])

        def start(self):
            self.part(NP - 1).start()

        def wait(self):
            for q in range(NP):
                self.part(q).wait()

    if MAN:
        for cp in wcopies:
            cp.start()
    head_copy().start()
    in_copy(0).start()
    if _env("K_D1", "1") == "0":
        in_copy(1).start()

    def column(row):
        row = jnp.concatenate([row, jnp.zeros((1, 128 - C), f32)], axis=1)
        return jnp.broadcast_to(row, (128, 128)).T[:C, :]

    def prepare():
        if MAN:
            for cp in wcopies:
                cp.wait()
        for t in range(9):
            dwb[t] = column(dw_ref[t // 3, pl.ds(t % 3, 1), :].astype(f32))
        w1 = w1_ref[...].astype(f32)
        w1 = w1 - jnp.sum(w1, axis=0, keepdims=True) * (1.0 / C)
        b1 = b1_ref[...].astype(f32) * _S
        b1h = b1.astype(bf16).astype(f32)
        b1l = b1 - b1h
        rows = jax.lax.broadcasted_iota(jnp.int32, (128 - C, E), 0)
        ext = jnp.where(rows == 0, b1h, jnp.where(rows == 1, b1l, 0.0))
        w1full = jnp.concatenate([w1, ext], axis=0)
        w1e[...] = pltpu.bitcast(w1full.T.astype(bf16), u32)
        g = g_ref[...].astype(f32)
        gcol = column(g)
        b2b[...] = column(b2_ref[...].astype(f32) * g)
        w2t = w2t_ref[...].astype(f32)
        gfull = jnp.concatenate([gcol] * (E // 128), axis=1)
        w2e[...] = pltpu.bitcast((w2t * (gfull * (0.5 / _S))).astype(bf16), u32)
        prow = jax.lax.broadcasted_iota(jnp.int32, (128 - C, W), 0)
        ones_rows = pltpu.bitcast(jnp.where(prow < 2, 1.0, 0.0).astype(bf16), u32)
        for s in range(SX):
            if XM == "b":
                XN[s][pl.ds(C // 2, 64 - C // 2), :] = ones_rows
            else:
                XN[s][pl.ds(C, 128 - C), :] = jnp.where(prow < 2, 1.0, 0.0)
        for ref in xs + XL + XR + XN + OUTS + sum(GS, []):
            ref[pl.ds(0, 8), pl.ds(0, 128)] = jnp.zeros((8, 128), ref.dtype)
        xs[-1 % U][...] = jnp.zeros((C, W), f32)
        if MODE == "H":
            XL[-1 % SH][...] = jnp.zeros((C, W), f32)
            XR[-1 % SH][...] = jnp.zeros((C, W), f32)
        xbuf[(NIT - 1) % NBI, U] = jnp.zeros((C, W), bf16)

        return b1l

    def tile(v):
        return jnp.concatenate([v] * NT, axis=1)

    def split(v):
        return [v[:, 128 * k:128 * (k + 1)] for k in range(NT)]

    class Row:
        pass

    DZ = _env("K_DZ", "")

    def dz(name, z, off, n):
        return pl.ds(pl.multiple_of(z + off, 8), n) if name in DZ else pl.ds(off, n)

    def cvt(r, islot, k, z):
        xs[r % U][dz("x", z, 0, C), :] = xbuf[islot, k].astype(f32)

    def shift_group(r, g, z):
        lane = jax.lax.broadcasted_iota(jnp.int32, (8, 128), 1)
        cs = dz("h", z, 8 * g, 8)
        x = split(xs[r % U][pl.ds(pl.multiple_of(z + 8 * g, 8), 8), :])
        for k in range(NT):
            lt = pltpu.roll(x[k], 1, 1)
            if k == 0:
                pltpu.store(XL[r % SH].at[cs, pl.ds(0, 128)], jnp.where(lane != 0, lt, 0.0))
            else:
                XL[r % SH][cs, pl.ds(128 * k, 128)] = lt
            if k < NT - 1:
                pltpu.store(XL[r % SH].at[cs, pl.ds(128 * k + 128, 128)], lt, mask=lane == 0)
        for k in reversed(range(NT)):
            rt = pltpu.roll(x[k], 127, 1)
            if k == NT - 1:
                pltpu.store(XR[r % SH].at[cs, pl.ds(128 * k, 128)], jnp.where(lane != 127, rt, 0.0))
            else:
                XR[r % SH][cs, pl.ds(128 * k, 128)] = rt
            if k > 0:
                pltpu.store(XR[r % SH].at[cs, pl.ds(128 * k - 128, 128)], rt, mask=lane == 127)

    def conv_group(st, g):
        r = st.r
        cs = pl.ds(8 * g, 8)
        if MODE == "V":
            lane = jax.lax.broadcasted_iota(jnp.int32, (8, 128), 1)
            m0 = lane == 0
            m127 = lane == 127
            x0 = xs[(r - 1) % U][cs, :]
            x1 = xs[r % U][cs, :]
            x2 = xs[(r + 1) % U][cs, :]
            t = []
            for j in range(3):
                pr = [tile(dwb[j, cs, :]) * x0, tile(dwb[3 + j, cs, :]) * x1, tile(dwb[6 + j, cs, :]) * x2]
                q = int(_env("K_TORD", "021")[j])
                t.append((pr[(q + 1) % 3] + pr[(q + 2) % 3]) + pr[q] if q != 2 else (pr[0] + pr[1]) + pr[2])
            lt = [pltpu.roll(v, 1, 1) for v in split(t[0])]
            rt = [pltpu.roll(v, 127, 1) for v in split(t[2])]
            lft = [jnp.where(m0, 0.0 if k == 0 else lt[k - 1], lt[k]) for k in range(NT)]
            rgt = [jnp.where(m127, 0.0 if k == NT - 1 else rt[k + 1], rt[k]) for k in range(NT)]
            lf, rg = jnp.concatenate(lft, axis=1), jnp.concatenate(rgt, axis=1)
            o = {"0": lambda: (lf + t[1]) + rg, "1": lambda: (lf + rg) + t[1], "2": lambda: (rg + t[1]) + lf}[_env("K_ASSOC", "2")]()
        else:
            t = []
            for i in range(3):
                q = r + i - 1
                t.append(tile(dwb[3 * i, cs, :]) * XL[q % SH][cs, :] + tile(dwb[3 * i + 1, cs, :]) * xs[q % U][cs, :]
                         + tile(dwb[3 * i + 2, cs, :]) * XR[q % SH][cs, :])
            o = (t[0] + t[1]) + t[2]
        GA = int(_env("K_GA", "0"))
        for q in range(int(_env("K_SRT", "0")) if g > 0 else 0):
            SR[q, cs, :] = st.s1
            st.s1 = SR[q, pl.ds(pl.multiple_of(st.z + 8 * g, 8), 8), :]
        if g == GA and GA:
            st.a = split(st.s1) + split(st.s2)
            for q in range(int(_env("K_DA", "0"))):
                st.a = [pltpu.roll(v, st.z, 1) for v in st.a]
            if _env("K_AM", "0") == "0":
                st.s1 = jnp.concatenate(st.a[:NT], axis=1) + o
                st.s2 = jnp.concatenate(st.a[NT:], axis=1) + o * o
            else:
                st.sa1 = jnp.concatenate(st.a[:NT], axis=1)
                st.sa2 = jnp.concatenate(st.a[NT:], axis=1)
                st.s1 = o
                st.s2 = o * o
        elif g == 0:
            st.s1 = o
            st.s2 = o * o
        else:
            st.s1 = st.s1 + o
            st.s2 = st.s2 + o * o
        if g == G - 1 and GA and _env("K_AM", "0") != "0":
            st.s1 = st.s1 + st.sa1
            st.s2 = st.s2 + st.sa2
        OUTS[r % NO][cs, :] = o

    def bcast_rows(v):
        return jnp.concatenate([jnp.broadcast_to(v[k:k + 1, :], (8, 128)) for k in range(NT)], axis=1)

    def stats(st):
        stats_a(st)
        stats_b(st)

    def stats_a(st):
        for k, v in enumerate(split(st.s1) + split(st.s2)):
            ST[pl.ds(k, 8, stride=8), :] = v

    def stats_b(st):
        st.ds = [OUTS[st.r % NO][pl.ds(pl.multiple_of(st.z + 8 * g, 8), 8), :] for g in range(G)]
        l = [ST[pl.ds(8 * j, 8), :] for j in range(8)]
        if _env("K_TREE", "0") == "1":
            s = ((l[0] + l[1]) + (l[2] + l[3])) + ((l[4] + l[5]) + (l[6] + l[7]))
        elif _env("K_TREE", "0") == "2":
            s = (((l[0] + l[1]) + l[2]) + l[3]) + (((l[4] + l[5]) + l[6]) + l[7])
        else:
            s = functools.reduce(lambda a, b: a + b, l)
        s = s * (1.0 / C)
        var = pltpu.roll(s, 4, 0) - s * s
        for q in range(int(_env("K_DLAT", "0"))):
            var = pltpu.roll(var, st.z, 1)
        for q in range(int(_env("K_DM", "7"))):
            var = jnp.maximum(var, -1.0 - q) + 0.0 if q % 2 else -jnp.minimum(-var, 1.0 + q)
        for q in range(int(_env("K_RT", "0"))):
            RT[q][1] = var
            var = RT[q][st.z + 1]
        ve = jnp.maximum(var, 0.0) + 1e-5
        rs = jax.lax.rsqrt(ve)
        st.mk2 = s
        MK = _env("K_MK", "")
        st.mk = {"": None, "v": ve, "r": rs, "s": s}[MK]
        rs = rs * _S
        for q in range(int(_env("K_DN", "1"))):
            rs = jnp.maximum(rs, -1.0 - q) if q % 2 else jnp.minimum(rs, 1e30 + q * 1e29)
        st.rstd = bcast_rows(rs)

    def normalize(st):
        ds = st.ds
        if (st.mk is not None and str(st.r % U) not in _env('K_MKX', '')) or _env("K_OD", "0") == "1":
            O = OUTT[st.r % NO]
            if st.mk is not None:
                O[1, pl.ds(0, 8), pl.ds(0, 128)] = st.mk
            n0 = int(_env("K_MK0", "0"))
            ds = ds[:n0] + [O[st.z, pl.ds(8 * g, 8), :] for g in range(n0, G)]
        xn = jnp.concatenate([d * st.rstd for d in ds], axis=0)
        if XM == "f":
            XN[st.r % SX][pl.ds(0, C), :] = xn
            return
        pk = pltpu.bitcast(xn.astype(bf16), u32)
        XN[st.r % SX][dz('n', st.z, 0, C // 2), :] = pk
        if str(st.k) in _env("K_PRI", "-"):
            for q in range(int(_env("K_PN", "1"))):
                v = (pk[C // 2 - 8:, :128] if _env("K_PW", "n") == "n" else st.mk2) if q == 0 else v
                v = pltpu.roll(v, 1, 1)
            SR[0, pl.ds(0, 8), pl.ds(0, 128)] += v if v.dtype == f32 else pltpu.bitcast(v, f32)

    def mm1(st, r):
        rhs = pltpu.bitcast(XN[r % SX][...], bf16) if XM == 'b' else XN[r % SX][...]
        st.y = jnp.dot(pltpu.bitcast(w1e[...], bf16), rhs, preferred_element_type=f32)

    def gelu_store(st, r, j, z):
        y = st.y[16 * j:16 * (j + 1), :]
        u = y * (y * y + _A)
        gl = y * jnp.tanh(u) + y if _env("K_GV", "1") == "0" else (jnp.tanh(u) + 1.0) * y
        e, jj = divmod(j, 8)
        if GM[e] == "f":
            GS[r % SG][e][pl.ds(16 * jj, 16), :] = gl
        else:
            GS[r % SG][e][dz('g', z, 8 * jj, 8), :] = pltpu.bitcast(gl.astype(bf16), u32)

    def mm2_lane(st, r, kk):
        acc = None
        ls = pl.ds(128 * kk, 128)
        for e in [int(c) for c in _env("K_EO", "012")]:
            gt = pltpu.bitcast(GS[r % SG][e][:, ls], bf16) if GM[e] == "b" else GS[r % SG][e][:, ls]
            w = pltpu.bitcast(w2e[:, pl.ds(128 * e, 128)], bf16)
            o = jnp.dot(w, gt, preferred_element_type=f32)
            prev = acc
            acc = o if acc is None else acc + o
        if kk == 0:
            st.accs = []
        xr = xs[r % U][:, ls]
        st.accs.append({"0": lambda: acc + (b2b[...] + xr), "1": lambda: (acc + b2b[...]) + xr, "2": lambda: o + (prev + (b2b[...] + xr))}[_env("K_EPI", "0")]())

    def epi_pair(st, oslot, k, p):
        v = jnp.concatenate(st.accs[2 * p:2 * p + 2], axis=1)
        obuf[oslot, k, :, pl.ds(256 * p, 256)] = v.astype(bf16)

    def phase(p, k, islot, irow, oslot, z, lo=-10 ** 9, i=None):
        A = Row()
        A.r = p - LA
        A.z, A.k = z, k
        B = Row()
        Cc = Row()
        rb, rc = p - LA - LB, p - OFF
        defer = DEFER and (k == U - 1 or (k is None and p == OFF - 1))
        prog = PROG
        if DEFER and k == 0:
            ps = _prog(_env("K_PROG0", "N," + ",".join(PROG)))
            prog = ps
        for tok in prog:
            t, a = tok[0], (int(tok[1:]) if len(tok) > 1 else None)
            if t == "o" and i is not None and (k + 1) % UP == 0 and not (OH and k == U - 1):
                out_copy(i).part(k // UP).start()
            elif t == "i" and i is not None and k % UI == int(_env("K_LK", "7")):
                in_copy(i + 2).part(k // UI).start()
            elif t == "w" and i is not None and k % UI == 0:
                in_copy(i).part(k // UI).wait()
            elif t == "c" and A.r >= lo:
                conv_group(A, a)
            elif t == "s" and A.r >= lo:
                stats_a(A) if defer else stats(A)
            elif t == "n" and A.r >= lo:
                if not defer:
                    normalize(A)
            elif t == "N":
                D = Row()
                D.r, D.z, D.k = A.r - 1, z, None
                stats_b(D)
                normalize(D)
            elif t == "m" and rc >= lo:
                mm2_lane(Cc, rc, a)
                if a % 2 == 1:
                    epi_pair(Cc, oslot, k, a // 2)
            elif t == "M" and rb >= lo:
                mm1(B, rb)
            elif t == "g" and rb >= lo:
                gelu_store(B, rb, a, z)
            elif t == "r" and MODE == "H" and p - LR >= lo:
                shift_group(p - LR, a, z)
            elif t == "v":
                cvt(p, islot, irow, z)

    head_copy().wait()
    if _env("K_LATE", "2") == "1":
        in_copy(2).start()
    one = None
    del one

    LW = _env("K_LW", "")
    if "i" in LW:
        in_copy(0).wait()
    OH = int(_env("K_OH", "0"))
    WI = int(_env('K_WI', '0'))
    if _env("K_D1", "1") == "1":
        in_copy(1).start()
    NREP = int(_env("K_NREP", "1"))

    def loop_body(i0, _):
        for rep in range(NREP):
            i = i0 * NREP + rep
            islot = i % NBI
            oslot = i % NBO
            if OH:
                @pl.when(i >= 1)
                def _():
                    out_copy(i - 1).start()
            if "i" not in LW and not WI:
                in_copy(i).wait()
            if "b" in BARR:
                @pl.when(i > 1000)
                def _():
                    xbuf[islot] = jnp.zeros((U + 1, C, W), bf16)
            if _env("K_LATE", "2") == "0":
                in_copy(i + 2).start()

            if "o" not in LW:
                @pl.when(i >= NBO)
                def _():
                    out_copy(i - NBO).wait()

            z = (i >> 21) * 8
            delta = jnp.maximum(OFF + i * U - (H - U), 0)
            for k in range(U):
                if WI and k % UI == 0 and _env("K_WP", "0") == "0":
                    in_copy(i).part(k // UI).wait()
                phase(OFF + k, k, islot, jnp.minimum(k + delta, U), oslot, z, i=i)
                if (k + 1) % UP == 0 and k + 1 < U and 'o' not in PROG:
                    out_copy(i).part(k // UP).start()
                if _env("K_LATE", "2") == "2" and k % UI == int(_env("K_LK", "7")):
                    in_copy(i + 2).part(k // UI).start()
            if 'o' not in PROG and not OH:
                out_copy(i).start()
            if _env("K_LATE", "2") == "1":
                in_copy(i + 3).start()
            if "i" in LW:
                in_copy(i + 1).wait()
            if "o" in LW:
                @pl.when(i + 1 >= NBO)
                def _():
                    out_copy(i + 1 - NBO).wait()
        return None

    def fill(i):
        z = (i >> 21) * 8
        for p in range(OFF):
            phase(p, None, NBI - 1, p, None, z, lo=0)
        return None

    if "g" in BARR:
        pid = pl.program_id(0)
    elif "d" in BARR:
        bits = pltpu.bitcast(dw_ref[0, pl.ds(0, 2), :].astype(f32), jnp.int32)
        pid = (jnp.max(bits) & 1) >> 1
    else:
        b1l = prepare()
        bits = pltpu.bitcast(b1l[:, :128], jnp.int32)
        pid = jnp.max(bits & 1) >> 1

    @pl.when(pid == 0)
    def _():
        if "g" in BARR or "d" in BARR:
            prepare()
        fill(pid)
    jax.lax.fori_loop(0, NIT // NREP, loop_body, None)
    if _env("K_PRI", "-") != "-":
        @pl.when(jnp.max(pltpu.bitcast(SR[0, pl.ds(0, 8), pl.ds(0, 128)], jnp.int32) & 1) > 1)
        def _():
            xbuf[0, 0] = jnp.zeros((C, W), bf16)
    if OH:
        out_copy(NIT - 1).start()
    if "i" not in LW:
        in_copy(NIT).wait()
    in_copy(NIT + 1).wait()
    if _env("K_LATE", "2") == "1":
        in_copy(NIT + 2).wait()
    for i in range(NIT - NBO + ("o" in LW), NIT):
        out_copy(i).wait()


def isem_one(r):
    return 0


@jax.jit
def pallas_standalone__modern_conv_block_convnext__vision_kernel(x, dw, w1, b1, w2, b2, gamma):
    B, H, W, C = x.shape
    E = w1.shape[1]
    xt = jnp.transpose(x, (0, 1, 3, 2)).reshape(B * H, C, W)
    w2t = w2.T
    kern = functools.partial(_kernel, H=H, C=C, W=W, E=E)
    man = _env("K_MAN", "1") == "1"
    ws = (dw, w1, b1.reshape(1, E), w2t, b2.reshape(1, C), gamma.reshape(1, C))
    vm = pl.BlockSpec(memory_space=pltpu.VMEM) if _env('K_VM', '1') == '1' else None
    out = pl.pallas_call(
        kern,
        grid=(1,),
        in_specs=[pl.BlockSpec(memory_space=pl.ANY), vm, vm, vm, vm, vm, vm] if not man else [pl.BlockSpec(memory_space=pl.ANY)] * 7,
        out_specs=pl.BlockSpec(memory_space=pl.ANY),
        out_shape=jax.ShapeDtypeStruct((H, C, W), x.dtype),
        scratch_shapes=[
            pltpu.VMEM((NBI, U + 1, C, W), bf16),
            pltpu.VMEM((NBO, U, C, W), bf16),
            pltpu.VMEM((9, C, 128), f32),
            pltpu.VMEM((E // 2, 128), u32),
            pltpu.VMEM((C // 2, E), u32),
            pltpu.VMEM((C, 128), f32),
            pltpu.VMEM((64, 128), f32),
            pltpu.SemaphoreType.DMA((NBI, int(_env("K_NI", "2")))),
            pltpu.SemaphoreType.DMA((NBO, int(_env("K_NP", "4")))),
        ] + [pltpu.VMEM((C, W), f32)] * U
          + [pltpu.VMEM((64, W), u32) if XM == 'b' else pltpu.VMEM((128, W), f32)] * SX
          + [pltpu.VMEM((64, W), u32) if m == 'b' else pltpu.VMEM((128, W), f32) for m in GM] * SG
          + [pltpu.VMEM((C, W), f32)] * NO
          + [pltpu.VMEM((C, W), f32)] * (2 * SH) + [pltpu.VMEM((2, 8, 128), f32)] * 8
          + ([pltpu.VMEM(w.shape, w.dtype) for w in ws] + [pltpu.SemaphoreType.DMA((6,))] if man else []),
        compiler_params=pltpu.CompilerParams(vmem_limit_bytes=100 * 1024 * 1024, disable_bounds_checks=bool(int(_env("K_DBC", "1")))),
    )(xt, *ws)
    return jnp.transpose(out.reshape(B, H, C, W), (0, 1, 3, 2))
```

```python
import functools
import math

import jax
import jax.numpy as jnp
from jax.experimental import pallas as pl
from jax.experimental.pallas import tpu as pltpu

_C1 = math.sqrt(2.0 / math.pi)
_C2 = _C1 * 0.044715
_S = _C2 ** (1.0 / 3.0)
_A = _C1 / _S

U = 32
UO = 4
NB = 4
LA, LB, OFF = 2, 3, 6
SX, SG, NO = 2, 4, 2

f32 = jnp.float32
bf16 = jnp.bfloat16
u32 = jnp.uint32


def _kernel(x_hbm, dw_hbm, w1_hbm, b1_hbm, w2t_hbm, b2_hbm, g_hbm, o_hbm,
            xbuf, obuf, dwb, w1e, w2e, b2b, st, isem, osem, *rest, H, C, W, E):
    rest = list(rest)

    def take(n):
        out = rest[:n]
        del rest[:n]
        return out

    xs = take(U)
    xn = take(SX)
    gs = [take(3) for _ in range(SG)]
    conv = take(NO)
    dw_ref, w1_ref, b1_ref, w2t_ref, b2_ref, g_ref, wsem = take(7)
    NT, G, NIT = W // 128, C // 8, H // U

    wcopies = [pltpu.make_async_copy(a, b, wsem.at[j]) for j, (a, b) in enumerate(zip(
        (dw_hbm, w1_hbm, b1_hbm, w2t_hbm, b2_hbm, g_hbm), (dw_ref, w1_ref, b1_ref, w2t_ref, b2_ref, g_ref)))]
    head_copy = pltpu.make_async_copy(x_hbm.at[pl.ds(0, OFF)], xbuf.at[NB - 1, pl.ds(0, OFF)], isem.at[NB - 1])

    def in_copy(ch):
        start = jnp.minimum(OFF + ch * U, H - U)
        slot = ch % NB
        return pltpu.make_async_copy(x_hbm.at[pl.ds(start, U)], xbuf.at[slot, pl.ds(0, U)], isem.at[slot])

    def out_copy(i, q):
        slot = i % NB
        return pltpu.make_async_copy(obuf.at[slot, pl.ds(q * UO, UO)], o_hbm.at[pl.ds(i * U + q * UO, UO)],
                                     osem.at[slot, q])

    for cp in wcopies:
        cp.start()
    head_copy.start()
    in_copy(0).start()

    def prepare_weights():
        for cp in wcopies:
            cp.wait()

        def column(row):
            row = jnp.concatenate([row, jnp.zeros((1, 128 - C), f32)], axis=1)
            return jnp.broadcast_to(row, (128, 128)).T[:C, :]

        for t in range(9):
            dwb[t] = column(dw_ref[t // 3, pl.ds(t % 3, 1), :].astype(f32))
        w1 = w1_ref[...].astype(f32)
        w1 = w1 - jnp.sum(w1, axis=0, keepdims=True) * (1.0 / C)
        b1 = b1_ref[...].astype(f32) * _S
        b1h = b1.astype(bf16).astype(f32)
        rows = jax.lax.broadcasted_iota(jnp.int32, (128 - C, E), 0)
        ext = jnp.where(rows == 0, b1h, jnp.where(rows == 1, b1 - b1h, 0.0))
        w1e[...] = pltpu.bitcast(jnp.concatenate([w1, ext], axis=0).T.astype(bf16), u32)
        g = g_ref[...].astype(f32)
        gcol = column(g)
        b2b[...] = column(b2_ref[...].astype(f32) * g)
        gfull = jnp.concatenate([gcol] * (E // 128), axis=1)
        w2e[...] = pltpu.bitcast((w2t_ref[...].astype(f32) * (gfull * (0.5 / _S))).astype(bf16), u32)
        prow = jax.lax.broadcasted_iota(jnp.int32, (128 - C, W), 0)
        ones_rows = pltpu.bitcast(jnp.where(prow < 2, 1.0, 0.0).astype(bf16), u32)
        for s in range(SX):
            xn[s][pl.ds(C // 2, 64 - C // 2), :] = ones_rows
        for ref in xs + xn + conv + sum(gs, []):
            ref[pl.ds(0, 8), pl.ds(0, 128)] = jnp.zeros((8, 128), ref.dtype)
        xs[-1 % U][...] = jnp.zeros((C, W), f32)
        xbuf[(NIT - 1) % NB, U] = jnp.zeros((C, W), bf16)

    def tile(v):
        return jnp.concatenate([v] * NT, axis=1)

    def split(v):
        return [v[:, 128 * k:128 * (k + 1)] for k in range(NT)]

    def conv_row(r):
        s1 = s2 = None
        for g in range(G):
            lane = jax.lax.broadcasted_iota(jnp.int32, (8, 128), 1)
            m0, m127 = lane == 0, lane == 127
            cs = pl.ds(8 * g, 8)
            x = [xs[(r + q) % U][cs, :] for q in (-1, 0, 1)]
            t = []
            for j in range(3):
                pr = [tile(dwb[3 * q + j, cs, :]) * x[q] for q in range(3)]
                t.append((pr[1] + pr[2]) + pr[0] if j == 0 else (pr[0] + pr[1]) + pr[2])
            lt = [pltpu.roll(v, 1, 1) for v in split(t[0])]
            rt = [pltpu.roll(v, 127, 1) for v in split(t[2])]
            lf = [jnp.where(m0, 0.0 if k == 0 else lt[k - 1], lt[k]) for k in range(NT)]
            rg = [jnp.where(m127, 0.0 if k == NT - 1 else rt[k + 1], rt[k]) for k in range(NT)]
            o = (jnp.concatenate(lf, axis=1) + jnp.concatenate(rg, axis=1)) + t[1]
            s1 = o if g == 0 else s1 + o
            s2 = o * o if g == 0 else s2 + o * o
            conv[r % NO][cs, :] = o
        return split(s1) + split(s2)

    def normalize(r, z):
        ds = [conv[r % NO][pl.ds(pl.multiple_of(z + 8 * g, 8), 8), :] for g in range(G)]
        s = functools.reduce(lambda a, b: a + b, [st[pl.ds(8 * j, 8), :] for j in range(8)])
        s = s * (1.0 / C)
        var = pltpu.roll(s, 4, 0) - s * s
        for q in range(7):
            var = jnp.maximum(var, -1.0 - q) + 0.0 if q % 2 else -jnp.minimum(-var, 1.0 + q)
        rs = jnp.minimum(jax.lax.rsqrt(jnp.maximum(var, 0.0) + 1e-5) * _S, 1e30)
        rs = jnp.concatenate([jnp.broadcast_to(rs[k:k + 1, :], (8, 128)) for k in range(NT)], axis=1)
        v = jnp.concatenate([d * rs for d in ds], axis=0)
        xn[r % SX][pl.ds(0, C // 2), :] = pltpu.bitcast(v.astype(bf16), u32)

    def mlp1(r):
        y = jnp.dot(pltpu.bitcast(w1e[...], bf16), pltpu.bitcast(xn[r % SX][...], bf16),
                    preferred_element_type=f32)

        def gelu(j):
            v = y[16 * j:16 * (j + 1), :]
            v = (jnp.tanh(v * (v * v + _A)) + 1.0) * v
            gs[r % SG][j // 8][pl.ds(8 * (j % 8), 8), :] = pltpu.bitcast(v.astype(bf16), u32)
        return gelu

    def mlp2(r, out):
        res = []
        for k in range(NT):
            ls = pl.ds(128 * k, 128)
            acc = None
            for e in (1, 0, 2):
                o = jnp.dot(pltpu.bitcast(w2e[:, pl.ds(128 * e, 128)], bf16),
                            pltpu.bitcast(gs[r % SG][e][:, ls], bf16), preferred_element_type=f32)
                acc = o if acc is None else acc + o
            res.append(acc + (b2b[...] + xs[r % U][:, ls]))
            if k % 2:
                out[:, pl.ds(128 * (k - 1), 256)] = jnp.concatenate(res[-2:], axis=1).astype(bf16)

    def phase(p, src, z, out=None, pending=False, defer=False):
        if pending:
            normalize(p - LA - 1, z)
        if out is not None:
            mlp2(p - OFF, out)
        xs[p % U][...] = src[...].astype(f32)
        gelu = mlp1(p - LB) if p >= LB else None
        if p >= LA:
            sums = conv_row(p - LA)
        if gelu is not None:
            for j in range(E // 16):
                gelu(j)
        if p >= LA:
            for k, v in enumerate(sums):
                st[pl.ds(k, 8, stride=8), :] = v
            if not defer:
                normalize(p - LA, z)

    head_copy.wait()
    pid = pl.program_id(0)

    @pl.when(pid == 0)
    def _():
        prepare_weights()
        for p in range(OFF):
            phase(p, xbuf.at[NB - 1, p], (pid >> 21) * 8, defer=p == OFF - 1)

    in_copy(1).start()

    def loop_body(i, _):
        slot = i % NB
        in_copy(i).wait()

        @pl.when(i >= NB)
        def _():
            for q in range(U // UO):
                out_copy(i - NB, q).wait()

        z = (i >> 21) * 8
        delta = jnp.maximum(OFF + i * U - (H - U), 0)
        for k in range(U):
            phase(OFF + k, xbuf.at[slot, jnp.minimum(k + delta, U)], z, obuf.at[slot, k],
                  pending=k == 0, defer=k == U - 1)
            if k % UO == UO - 1:
                out_copy(i, k // UO).start()
            if k == 2:
                in_copy(i + 2).start()

    jax.lax.fori_loop(0, NIT, loop_body, None)
    in_copy(NIT).wait()
    in_copy(NIT + 1).wait()
    for i in range(NIT - NB, NIT):
        for q in range(U // UO):
            out_copy(i, q).wait()


@jax.jit
def pallas_standalone__modern_conv_block_convnext__vision_kernel(x, dw, w1, b1, w2, b2, gamma):
    B, H, W, C = x.shape
    E = w1.shape[1]
    assert B == 1 and H % U == 0 and H // U >= NB and W == 512
    xt = jnp.transpose(x, (0, 1, 3, 2)).reshape(H, C, W)
    ws = (dw, w1, b1.reshape(1, E), w2.T, b2.reshape(1, C), gamma.reshape(1, C))
    out = pl.pallas_call(
        functools.partial(_kernel, H=H, C=C, W=W, E=E),
        grid=(1,),
        in_specs=[pl.BlockSpec(memory_space=pl.ANY)] * 7,
        out_specs=pl.BlockSpec(memory_space=pl.ANY),
        out_shape=jax.ShapeDtypeStruct((H, C, W), x.dtype),
        scratch_shapes=[
            pltpu.VMEM((NB, U + 1, C, W), bf16),
            pltpu.VMEM((NB, U, C, W), bf16),
            pltpu.VMEM((9, C, 128), f32),
            pltpu.VMEM((E // 2, 128), u32),
            pltpu.VMEM((C // 2, E), u32),
            pltpu.VMEM((C, 128), f32),
            pltpu.VMEM((64, 128), f32),
            pltpu.SemaphoreType.DMA((NB,)),
            pltpu.SemaphoreType.DMA((NB, U // UO)),
        ] + [pltpu.VMEM((C, W), f32)] * U
          + [pltpu.VMEM((64, W), u32)] * (SX + 3 * SG)
          + [pltpu.VMEM((C, W), f32)] * NO
          + [pltpu.VMEM(w.shape, w.dtype) for w in ws]
          + [pltpu.SemaphoreType.DMA((6,))],
        compiler_params=pltpu.CompilerParams(vmem_limit_bytes=100 * 1024 * 1024, disable_bounds_checks=True),
    )(xt, *ws)
    return jnp.transpose(out.reshape(B, H, C, W), (0, 1, 3, 2))
```
